```python
import os as _os
_os.environ.setdefault("JAX_PLATFORMS", "cpu")
import jax
import jax.numpy as jnp

def _softmax(x, axis=-1):
    return jax.nn.softmax(x, axis=axis)
def _gelu(x):
    return jax.nn.gelu(x, approximate=True)
def _silu(x):
    return jax.nn.silu(x)
def _sigmoid(x):
    return jax.nn.sigmoid(x)
def _layernorm(x, axis=-1, eps=1e-5):
    m = jnp.mean(x, axis=axis, keepdims=True)
    v = jnp.var(x, axis=axis, keepdims=True)
    return (x - m) / jnp.sqrt(v + eps)
def _scatter_add(tgt, idx, src, axis=0):
    return tgt.at[idx].add(src)
def _segment_sum(src, seg, n):
    return jax.ops.segment_sum(src, seg, n)
class _Rng:
    def __init__(self, key):
        self._k = key
    def _next(self):
        self._k, sub = jax.random.split(self._k)
        return sub
    def normal(self, shape):
        return jax.random.normal(self._next(), shape, dtype=jnp.bfloat16)
    def randint(self, lo, hi, shape):
        return jax.random.randint(self._next(), shape, lo, hi, dtype=jnp.int32)
    def uniform(self, shape, lo=0.0, hi=1.0):
        return jax.random.uniform(self._next(), shape, jnp.bfloat16, lo, hi)
    def permutation(self, n):
        return jax.random.permutation(self._next(), n)


kernel_name = 'gated_mix__grouped_kv_mqa__glu_gated_reglu__prompt'

def setup_inputs():
    _rng = _Rng(jax.random.key(int.from_bytes(__import__("os").urandom(4), "little")))
    _w = (lambda a: (lambda t: t.astype(jnp.bfloat16) if jnp.issubdtype(t.dtype, jnp.floating) else t)(jnp.asarray(a)))
    def _A_setup():
        B, S, D, H = 1, 2048, 640, 32
        Dh = D // H
        return {
            "x": _w((lambda *s: _rng.normal(s) * 0.05)(B, S, D)),
            "wq": _w((lambda *s: _rng.normal(s) * 0.2)(D, H * Dh)),
            "wk": _w((lambda *s: _rng.normal(s) * 0.2)(D, Dh)),
            "wv": _w((lambda *s: _rng.normal(s) * 0.05)(D, Dh)),
            "wo": _w((lambda *s: _rng.normal(s) * 0.05)(H * Dh, D)),
        }
    _A_in = _A_setup()

    def _B_setup():
        B, S, D, F = 1, 2048, 640, 1536
        return {
            "x": _w((lambda *s: _rng.normal(s) * 0.05)(B, S, D)),
            "W_gate": _w((lambda *s: _rng.normal(s) * 0.4)(D, F) * (2.0 / D) ** 0.5),
            "W_up": _w((lambda *s: _rng.normal(s) * 0.4)(D, F) * (2.0 / D) ** 0.5),
            "W_down": _w((lambda *s: _rng.normal(s) * 0.4)(F, D) * (1.0 / F) ** 0.5),
        }
    _B_in = _B_setup()

    return {
        "A_x": _A_in["x"],
        "A_wq": _A_in["wq"],
        "A_wk": _A_in["wk"],
        "A_wv": _A_in["wv"],
        "A_wo": _A_in["wo"],
        "B_x": _B_in["x"],
        "B_W_gate": _B_in["W_gate"],
        "B_W_up": _B_in["W_up"],
        "B_W_down": _B_in["W_down"],
        "gate_w": _w((lambda *s: _rng.normal(s) * 0.05)(640) * 16.0),
    }

def reference(A_x, A_wq, A_wk, A_wv, A_wo, B_x, B_W_gate, B_W_up, B_W_down, gate_w):
    def _A_ref(x, wq, wk, wv, wo):
        B, S, D = x.shape
        H = 32
        Dh = D // H
        q = (lambda x, *d: x.transpose(*d))((x @ wq).reshape(B, S, H, Dh), 0, 2, 1, 3)
        k = x @ wk
        v = x @ wv
        scores = jnp.einsum("bhqd,bkd->bhqk", q, k) * (Dh ** -0.5)
        p = _softmax(scores, axis=-1)
        o = jnp.einsum("bhqk,bkd->bhqd", p, v)
        return (lambda x, *d: x.transpose(*d))(o, 0, 2, 1, 3).reshape(B, S, H * Dh) @ wo

    def _B_ref(x, W_gate, W_up, W_down):
        gate = jnp.einsum("bsd,df->bsf", x, W_gate)
        up = jnp.einsum("bsd,df->bsf", x, W_up)
        gate = gate * (lambda x, dt: x.astype(dt))(gate > 0, gate.dtype)
        h = gate * up
        return jnp.einsum("bsf,fd->bsd", h, W_down)

    x = A_x
    g = _sigmoid((x * gate_w).sum(-1, keepdims=True))
    a = _A_ref(x, A_wq, A_wk, A_wv, A_wo)
    b = _B_ref(x, B_W_gate, B_W_up, B_W_down)
    return g * a + (1 - g) * b
```

```python
import functools
import math

import jax
import jax.numpy as jnp
from jax import lax
import jax.experimental.pallas as pl
import jax.experimental.pallas.tpu as pltpu

S, D, H, DH, F = 2048, 640, 32, 20, 1536
T = 128
NB = S // T
NSET = H // 4
VR = 24
NVMAX = 32
QSCALE = DH ** -0.5 * math.log2(math.e)
L_LO, L_HI = 2.0 ** -32, 2.0 ** 64
LAT = 127

NP = 8
K0 = 0
V0 = K0 + 4 * 64
P0 = V0 + 4 * VR
X0 = P0 + NP * 64
H0 = X0 + 2 * 64
O0 = H0 + 3 * 64
G0 = O0 + 2 * 64
A0 = G0 + T
J0 = A0 + 2 * T
SP_ROWS = J0 + NVMAX

BF, F32 = jnp.bfloat16, jnp.float32
NT = (((1,), (1,)), ((), ()))

DEFAULT = dict(nset=8, period=58.0, t0=200, skew=1, npl=4, parts=(20,), xlat=12, dur=1.0, tick=16, pre=32, j0=14, gk=16, gh=2, margin=8, la=2, slack=48,
               lead=40, otlag=300, xsplit=(256, 768, 1024), dma=0)


def _at(base, height, n, r=0):
    return base + (n // 4) * height + r, (n % 4) * T


def _dot(a, b):
    return jnp.dot(a, b, preferred_element_type=F32)


def _round(x):
    return x.astype(BF).astype(F32)


def _plan(cfg):
    nset, la, slack, lead = cfg["nset"], cfg["la"], cfg["slack"], cfg["lead"]
    gk, gh = cfg["gk"], cfg["gh"]
    nsteps = nset * NB
    jobs = []
    for G in range(F // 256):
        jobs += [("gu_b", G)] + [("gu_a", G, t) for t in range(4)]
        if G in (2, 4):
            jobs += [("down", G // 2 - 1, n) for n in range(5)]
    jobs += [("down", 2, n) for n in range(5)] + [("oproj", n) for n in range(5)]
    jobs[1:1] = [("olast", 0), ("olast", 1)]
    if nset < NSET:
        jobs = jobs[cfg["j0"]:cfg["j0"] + len(jobs) * nset // NSET]
    jobs, tail = jobs[:-la], jobs[-la:]
    slot = {(j + 1) * (nsteps - 2) // len(jobs): job for j, job in enumerate(jobs)}
    seq = []
    for i in range(nsteps + la):
        seq.append(("qk", i) if i < nsteps else tail[i - nsteps])
        if i in slot:
            seq.append(slot[i])
        if i >= la:
            seq.append(("pv", i - la))

    def height(job):
        if job[0] == "qk":
            return T - nv[job[1]]
        return VR if job[0] == "pv" else T // 4 if job == ("olast", 1) else T

    nv = [0] * nsteps
    per = 4 // gh
    for _ in range(8):
        now, p_load = 0, {}
        for job in seq:
            if job[0] == "pv":
                p_load[job[1]] = now - lead
            now += height(job)
        keys, t_free = [], cfg["t0"]
        for i in range(nsteps):
            if i >= NP:
                t_free = max(t_free, p_load[i - NP] + 1)
            ready = int((p_load[i] - cfg["margin"] - t_free) // cfg["period"]) + 1 - cfg["skew"]
            nv[i] = max(0, min(NVMAX // gk, ready // per)) * gk
            for k0 in range(0, nv[i], gk):
                keys.append((t_free, i, k0))
                t_free += per * cfg["period"]
    blocks = [(t + (n + 2 * n * cfg["skew"]) * cfg["period"], i, k0, n * gh)
              for t, i, k0 in keys for n in range(per)]

    events, now, t_pl, t_res = [], 0, {}, {}
    for job in seq:
        if job[0] == "pv":
            now = max(now, t_res[job[1]] + lead + 1)
        rows, step = height(job), 8 if job[0] == "pv" else 16
        full = T if job[0] == "olast" else rows
        events += [(now + r * rows // full, ("lhs", job, r)) for r in range(0, full, step)]
        events.append((now + (full - step) * rows // full, ("dot", job)))
        if job[0] == "pv":
            t_pl[job[1]] = now - lead
            np_ = cfg["npl"]
            events += [(now - lead + 32 * u // np_, ("p_load", job[1], np_ - 1 - u)) for u in range(np_)]
            if job[1] % NB == NB - 1:
                s = job[1] // NB
                events.append((now + rows + LAT + slack, ("norm", s)))
                for kt in range(4):
                    if (T * kt + T - 1) // (4 * DH) == s and nset == NSET:
                        events.append((now + rows + LAT + cfg["otlag"], ("otile", kt)))
        else:
            if job[0] != "qk":
                events += [(now + r + 8 + LAT + slack - cfg["pre"], ("pre", job, r))
                           for r in range(0, full, 16)]
            events += [(now + r + 8 + LAT + slack, ("res", job, r)) for r in range(0, full, 16)]
            if job[0] == "qk":
                t_res[job[1]] = events[-1][0]
        now += rows
    parts = cfg["parts"]
    for t, i, k0, t0 in blocks:
        t = min(t, t_pl[i] - 1)
        for u, d1 in enumerate(parts):
            early = 0 if d1 == DH else cfg["xlat"] + (DH - d1) * cfg["dur"] * cfg["period"] / DH
            events.append((t - early, ("vpu", i, k0, t0, parts[u - 1] if u else 0, d1)))
    events += [(-1, ("q_stage", 0)), (cfg["otlag"], ("otile", 4))]
    events += [(1200 * s, ("q_stage", s)) for s in range(1, nset)]
    events += [(8 + 16 * n, ("x_stage", kt)) for n, kt in enumerate((4, 0, 1, 2, 3))]
    tick = cfg["tick"]

    def key(e):
        t, ev = e
        return (t // tick, ev[0] in ("lhs", "dot", "p_load", "pre"), t) if tick else t

    return [e for _, e in sorted(events, key=key)], nv


def _kernel(cfg, x_hbm, wq_hbm, wkt_hbm, wvt_hbm, wo_hbm, wg_hbm, wu_hbm, wd_hbm, gw_hbm,
            out_hbm,
            x_v, wq_v, wkt_v, wvt_v, gw_v, wo_v, wg_v, wu_v, wd_v,
            qt_v, q_v, kb_v, sp_v, g_v, omg_v, ot_v, out_v,
            in_sem, out_sem):
    spans, lo = [], 0
    for n in cfg["xsplit"]:
        spans.append((lo, n))
        lo += n
    pairs = [(x_hbm.at[pl.ds(*sp)], x_v.at[pl.ds(*sp)]) for sp in spans]
    pairs += [(wq_hbm, wq_v), (wkt_hbm, wkt_v), (wvt_hbm, wvt_v), (gw_hbm, gw_v),
              (wg_hbm, wg_v), (wu_hbm, wu_v), (wd_hbm, wd_v), (wo_hbm, wo_v)]
    copies = [pltpu.make_async_copy(s, d, in_sem.at[i]) for i, (s, d) in enumerate(pairs)]
    x_copy, small, big = copies[:len(spans)], copies[len(spans):-4], copies[-4:]
    for c in x_copy[:1] + small:
        c.start()
    if cfg["dma"] == 0:
        for c in x_copy[1:] + big:
            c.start()
    for c in small:
        c.wait()
    if cfg["dma"] == 1:
        for c in x_copy[1:] + big:
            c.start()

    z4 = jnp.zeros((4, D), F32)
    wkv = jnp.concatenate(
        [wkt_v[...].astype(F32), z4, wvt_v[...].astype(F32), gw_v[...].astype(F32).reshape(1, D),
         z4[0:3]],
        axis=0).astype(BF)
    row = lax.broadcasted_iota(jnp.int32, (VR, T), 0)
    for (lo, n), copy in zip(spans, x_copy):
        copy.wait()
        kv = lax.dot_general(wkv, x_v[lo:lo + n, :], NT, preferred_element_type=F32)
        for c in range(lo // T, (lo + n) // T):
            rc = kv[:, c * T - lo:(c + 1) * T - lo]
            kn = jnp.concatenate([_round(rc[0:VR]), jnp.zeros((T - VR, T), F32)], axis=0).T
            kr, kc = _at(K0, 64, c)
            sp_v[kr:kr + 64, kc:kc + T] = pltpu.bitcast(kn.astype(BF), F32)
            for d in range(DH):
                kb = jnp.broadcast_to(kn[T - NVMAX:T, d:d + 1], (NVMAX, T))
                for j in range(NVMAX // 8):
                    kb_v[c, 8 * d:8 * d + 8, pl.ds(((j + d) % 4) * T, T)] = kb[8 * j:8 * j + 8]
            vg = rc[VR:2 * VR]
            vr, vc = _at(V0, VR, c)
            sp_v[vr:vr + VR, vc:vc + T] = jnp.where(
                row < DH, _round(vg), jnp.where(row == DH, 1.0, 0.0))
            g = jax.nn.sigmoid(vg[DH:DH + 1])
            g_v[c] = jnp.broadcast_to(g, (8, T))
            omg_v[c] = jnp.broadcast_to(1.0 - g, (T, T)).T
        for m0 in range(lo, lo + n, 2 * T):
            q = _dot(x_v[m0:m0 + 2 * T, :], wq_v[...])
            for c in range(m0 // T, m0 // T + 2):
                qs = _round(q[c * T - m0:(c + 1) * T - m0] * QSCALE).T
                qs = jnp.concatenate([qs, jnp.zeros((8, T), F32)], axis=0)
                for hd in range(H):
                    qt_v[c, (hd // 4) * VR:(hd // 4 + 1) * VR, (hd % 4) * T:(hd % 4 + 1) * T] = (
                        qs[hd * DH:hd * DH + VR])
    sp_v[A0:A0 + 2 * T, :] = jnp.zeros((2 * T, 4 * T), F32)
    ot_v[4 * T:5 * T, :] = jnp.zeros((T, T), F32)
    for c in big:
        c.wait()

    def out_copy(b):
        r0 = pl.multiple_of(b * T, T)
        return pltpu.make_async_copy(
            out_v.at[pl.ds(r0 + T, T)], out_hbm.at[pl.ds(r0, T)], out_sem.at[b])

    events, nv = _plan(cfg)
    gk, gh = cfg["gk"], cfg["gh"]

    def body(b, carry):
        l_min, l_max = carry
        r0 = pl.multiple_of(b * T, T)
        g = g_v[b, 0:1, :]
        z = pl.multiple_of(lax.shift_right_logical(b, 16) * 8, 8)
        st = {}

        def ld(rc, n, w=T):
            return sp_v[rc[0]:rc[0] + n, rc[1]:rc[1] + w]

        def put(rc, val):
            if val.dtype == BF:
                val = pltpu.bitcast(val, F32)
            sp_v[pl.ds(z + rc[0], val.shape[0]), rc[1]:rc[1] + val.shape[1]] = val

        def p_at(i, t, r):
            return _at(P0, 64, (i % NP) * 4 + t, r // 2)

        acc = None
        done = set()
        for ev in events:
            kind = ev[0]
            if kind == "vpu":
                i, k0, t0, d0, d1 = ev[1:]
                s, c = divmod(i, NB)
                g0 = (NVMAX - nv[i] + k0) // 8
                accs = st.setdefault((i, k0, t0), [None] * gh)
                for d in range(d0, d1):
                    kb = jnp.concatenate(
                        [kb_v[c, 8 * d:8 * d + 8, pl.ds(((g0 + j + d) % 4) * T, T)]
                         for j in range(gk // 8)], axis=0)
                    for t in range(gh):
                        term = kb * q_v[s * VR + d:s * VR + d + 1, (t0 + t) * T:(t0 + t + 1) * T]
                        accs[t] = accs[t] + term if d else term
                if d1 < DH:
                    for t in range(gh):
                        put((J0, (t0 + t) * T), accs[t])
                    continue
                for t in range(gh):
                    put(p_at(i, t0 + t, T - nv[i] + k0), jnp.exp2(accs[t]).astype(BF))
                done.add(("v", i, k0, t0))
                assert i < NP or ("pl", i - NP, 0) in done
            elif kind == "q_stage":
                q_v[ev[1] * VR:(ev[1] + 1) * VR, :] = qt_v[b, ev[1] * VR:(ev[1] + 1) * VR, :]
            elif kind == "x_stage":
                put(_at(X0, 64, ev[1]), x_v[pl.ds(r0, T), ev[1] * T:(ev[1] + 1) * T])
            elif kind == "p_load":
                i, u = ev[1:]
                assert all(("p", i, r) in done for r in range(0, T - nv[i], 16))
                assert all(("v", i, k0, t0) in done for k0 in range(0, nv[i], gk) for t0 in range(0, 4, gh))
                n = T // cfg["npl"]
                st.setdefault(("p", i), []).insert(0, ld(p_at(i, 0, u * n), n // 2, 4 * T))
                done.add(("pl", i, u))
            elif kind == "lhs":
                job, r = ev[1:]
                if job[0] == "qk":
                    v = ld(_at(K0, 64, job[1] % NB, r // 2), 8)
                elif job[0] == "pv":
                    v = ld(_at(V0, VR, job[1] % NB, r), 8)
                else:
                    base, tiles = {
                        "gu_b": (X0, [4]), "gu_a": (X0, range(4)),
                        "down": (H0, range(4 * job[1], 4 * job[1] + 4)),
                        "oproj": (O0, range(4)), "olast": (O0, [4])}[job[0]]
                    assert all((base, kt, r) in done for kt in tiles) or base == X0 or cfg["nset"] < NSET, job
                    v = ld(_at(base, 64, tiles[0], r // 2), 8, len(tiles) * T)
                st.setdefault(("lhs", job), []).append(v)
            elif kind == "dot":
                job = ev[1]
                lhs = jnp.concatenate(st.pop(("lhs", job)), axis=0)
                if job[0] == "pv":
                    o = _dot(lhs, pltpu.bitcast(jnp.concatenate(st.pop(("p", job[1])), axis=0), BF))
                    acc = o + acc if job[1] % NB else o
                    st["acc", job[1] // NB] = acc
                    continue
                lhs = pltpu.bitcast(lhs, BF)
                if job[0] == "qk":
                    s = job[1] // NB
                    lhs = lhs[:, 0:VR]
                    w = q_v[s * VR:(s + 1) * VR, :]
                elif job[0] == "gu_b":
                    c0 = job[1] * 256
                    w = jnp.concatenate(
                        [wg_v[512:640, c0:c0 + 256], wu_v[512:640, c0:c0 + 256]], axis=1)
                elif job[0] == "gu_a":
                    c0 = job[1] * 256 + (job[2] // 2) * T
                    w = (wg_v, wu_v)[job[2] % 2][0:512, c0:c0 + T]
                elif job[0] == "down":
                    w = wd_v[job[1] * 512:(job[1] + 1) * 512, job[2] * T:(job[2] + 1) * T]
                elif job[0] == "oproj":
                    w = wo_v[0:512, job[1] * T:(job[1] + 1) * T]
                else:
                    w = wo_v[512:640, (0, 512)[job[1]]:(512, 640)[job[1]]]
                st["y", job] = _dot(lhs, w)
            elif kind == "pre":
                job, r = ev[1:]
                if job[0] == "gu_a":
                    t = job[2]
                    src = [_at(G0, T, (t % 2) * 2 + t // 2, r)] + [_at(G0, T, t // 2, r)] * (t % 2)
                elif job[0] == "olast":
                    src = [_at(A0, T, m, r) for m in ((0, 1, 2, 3), (4,))[job[1]]]
                elif job[0] == "gu_b" or job[:2] == ("down", 0):
                    src = []
                else:
                    src = [_at(A0, T, job[-1], r)]
                assert all(rc in done for rc in src) or job[0] == "olast" or cfg["nset"] < NSET
                done.difference_update(src)
                st["pre", job, r] = [ld(rc, 16) for rc in src]
            elif kind == "res":
                job, r = ev[1:]
                y = st["y", job][r:r + 16]
                pre = st.pop(("pre", job, r), None)
                if job[0] == "qk":
                    put(p_at(job[1], 0, r), jnp.exp2(y).astype(BF))
                    done.add(("p", job[1], r))
                elif job[0] == "gu_b":
                    put((G0 + r, 0), y)
                    done.update(_at(G0, T, t, r) for t in range(4))
                elif job[0] == "gu_a":
                    G, t = job[1:]
                    rc = _at(G0, T, (t % 2) * 2 + t // 2, r)
                    y = y + pre[0]
                    if t % 2 == 0:
                        put(rc, jnp.maximum(y, 0.0) * omg_v[b, r:r + 16, :])
                        done.add(rc)
                    else:
                        kt = 2 * G + t // 2
                        put(_at(H0, 64, kt, r // 2), (pre[1] * y).astype(BF))
                        done.add((H0, kt, r))
                elif job[0] in ("down", "oproj"):
                    rc = _at(A0, T, job[-1], r)
                    put(rc, y + pre[0] if pre else y)
                    done.add(rc)
                else:
                    for m in ((0, 1, 2, 3), (4,))[job[1]]:
                        ym = y[:, (m % 4) * T:(m % 4 + 1) * T] + pre[m % 4]
                        out_v[pl.ds(r0 + r, 16), m * T:(m + 1) * T] = ym.astype(BF)
            elif kind == "norm":
                s = ev[1]
                for t in range(4):
                    a = st["acc", s][:, t * T:(t + 1) * T]
                    l = a[DH:DH + 1]
                    mag = jnp.maximum(jnp.maximum(jnp.abs(a[0:8]), jnp.abs(a[8:16])),
                                      jnp.abs(a[16:24]))
                    l_min = jnp.minimum(l_min, l)
                    l_max = jnp.maximum(l_max, mag)
                    ot_v[(4 * s + t) * DH:(4 * s + t + 1) * DH, :] = a[0:DH] * (g / l)
            elif kind == "otile":
                kt = ev[1]
                put(_at(O0, 64, kt), ot_v[kt * T:(kt + 1) * T, :].T.astype(BF))
                done.update((O0, kt, r) for r in range(0, T, 16))

        @pl.when(b > 0)
        def _():
            out_copy(b - 1).start()

        return l_min, l_max

    l_min, l_max = lax.fori_loop(
        0, NB, body, (jnp.full((1, T), 1.0, F32), jnp.full((8, T), 1.0, F32)))
    y = _dot(ot_v[4 * T:5 * T, :].T.astype(BF), wo_v[512:640, :])
    y += jnp.concatenate([sp_v[A0:A0 + T, :], sp_v[A0 + T:A0 + 2 * T, 0:T]], axis=1)
    out_v[S:S + T, :] = y.astype(BF)
    out_copy(NB - 1).start()
    safe = jnp.logical_and(jnp.min(l_min) >= L_LO, jnp.max(l_max) <= L_HI)
    for b in range(NB):
        out_copy(b).wait()

    @pl.when(jnp.logical_not(safe))
    def _():
        def blk(b, _):
            r0 = pl.multiple_of(b * T, T)
            g = g_v[b, 0:1, :]

            def head_set(s, _):
                q = qt_v[b, pl.ds(pl.multiple_of(s * VR, 8), VR), :]

                def scores(c):
                    kr, kc = _at(K0, 64, c)
                    return _dot(pltpu.bitcast(sp_v[kr:kr + 64, kc:kc + T], BF)[:, 0:VR], q)

                ss = [scores(c) for c in range(NB)]
                mx = functools.reduce(jnp.maximum, [jnp.max(y, axis=0, keepdims=True) for y in ss])
                a = None
                for c in range(NB):
                    vr, vc = _at(V0, VR, c)
                    o = _dot(sp_v[vr:vr + VR, vc:vc + T], jnp.exp2(ss[c] - mx).astype(BF))
                    a = o if a is None else o + a
                outs = [a[0:DH, t * T:(t + 1) * T] * (g / a[DH:DH + 1, t * T:(t + 1) * T])
                        for t in range(4)]
                ot_v[pl.ds(pl.multiple_of(s * 4 * DH, 8), 4 * DH), :] = jnp.concatenate(outs, axis=0)

            lax.fori_loop(0, NSET, head_set, None)
            xb = x_v[pl.ds(r0, T), :]
            h = (jnp.maximum(_dot(xb, wg_v[...]), 0.0) * _dot(xb, wu_v[...])).astype(BF)
            omg = jnp.concatenate([omg_v[b]] * 5, axis=1)
            y = _dot(ot_v[...].T.astype(BF), wo_v[...]) + omg * _dot(h, wd_v[...])
            out_v[pl.ds(r0, T), :] = y.astype(BF)

        lax.fori_loop(0, NB, blk, None)
        cp = pltpu.make_async_copy(out_v.at[pl.ds(0, S)], out_hbm, out_sem.at[0])
        cp.start()
        cp.wait()


def build(**kw):
    cfg = dict(DEFAULT)
    cfg.update(kw)
    flags = cfg.pop("flags", None)
    nv = _plan(cfg)[1]

    def fn(A_x, A_wq, A_wk, A_wv, A_wo, B_x, B_W_gate, B_W_up, B_W_down, gate_w):
        del B_x
        any_spec = pl.BlockSpec(memory_space=pl.ANY)
        out = pl.pallas_call(
            functools.partial(_kernel, cfg),
            out_shape=jax.ShapeDtypeStruct((S, D), A_x.dtype),
            in_specs=[any_spec] * 9,
            out_specs=any_spec,
            scratch_shapes=[
                pltpu.VMEM((S, D), BF), pltpu.VMEM((D, D), BF),
                pltpu.VMEM((DH, D), BF), pltpu.VMEM((DH, D), BF), pltpu.VMEM((D,), BF),
                pltpu.VMEM((D, D), BF), pltpu.VMEM((D, F), BF), pltpu.VMEM((D, F), BF),
                pltpu.VMEM((F, D), BF),
                pltpu.VMEM((NB, NSET * VR, 4 * T), F32),
                pltpu.VMEM((NSET * VR, 4 * T), F32),
                pltpu.VMEM((NB, DH * 8, 4 * T), F32),
                pltpu.VMEM((SP_ROWS, 4 * T), F32),
                pltpu.VMEM((NB, 8, T), F32),
                pltpu.VMEM((NB, T, T), F32),
                pltpu.VMEM((D, T), F32),
                pltpu.VMEM((S + T, D), BF),
                pltpu.SemaphoreType.DMA((8 + len(cfg["xsplit"]),)),
                pltpu.SemaphoreType.DMA((NB,)),
            ],
            compiler_params=pltpu.CompilerParams(vmem_limit_bytes=100 * 2 ** 20, flags=flags),
            name="mbk",
        )(A_x.reshape(S, D), A_wq, A_wk.T, A_wv.T, A_wo, B_W_gate, B_W_up, B_W_down,
          gate_w)
        return out.reshape(1, S, D)

    return jax.jit(fn)


pallas_gated_mix__grouped_kv_mqa__glu_gated_reglu__prompt_kernel = build(period=54, slack=56, parts=(10, 20))
```

```python
import math

import jax
import jax.numpy as jnp
from jax import lax
import jax.experimental.pallas as pl
import jax.experimental.pallas.tpu as pltpu

S, D, H, DH, F = 2048, 640, 32, 20, 1536
T = 128
NB = S // T
NSET = H // 4
NSTEP = NSET * NB
VR = 24
NV = 32
HD = DH // 2
QSCALE = DH ** -0.5 * math.log2(math.e)
L_LO, L_HI, V_HI = 2.0 ** -32, 2.0 ** 64, 2.0 ** 60
X_SPANS = ((0, 256), (256, 768), (1024, 1024))
VPU_BLOCKS = ((0, 0), (1, 2), (0, 2), (1, 0))

NP = 8
K0 = 0
V0 = K0 + 4 * 64
P0 = V0 + 4 * VR
X0 = P0 + NP * 64
H0 = X0 + 2 * 64
O0 = H0 + 3 * 64
G0 = O0 + 2 * 64
A0 = G0 + T
PV0 = A0 + 2 * T
J0 = PV0 + VR
SP_ROWS = J0 + 16

LAT = 127
SLACK = 56
LEAD = 40
AHEAD = 2
RATE = 3.78

BF, F32 = jnp.bfloat16, jnp.float32


def _at(base, height, n, r=0):
    return base + (n // 4) * height + r, (n % 4) * T


def _dot(a, b):
    return jnp.dot(a, b, preferred_element_type=F32)


def _unpack(ref, r0, r1, c0, c1):
    return pltpu.bitcast(ref[r0 // 2:r1 // 2, c0:c1], BF)


def _round(x):
    return x.astype(BF).astype(F32)


def _quarters(x, w):
    m = x.shape[0] // 4
    return jnp.concatenate([_dot(x[r * m:(r + 1) * m], w) for r in range(4)], axis=0)


def _last_rows_dot(x, w_ref):
    return jnp.concatenate([_dot(x, _unpack(w_ref, 512, D, 0, 512)),
                            _quarters(x, _unpack(w_ref, 512, D, 512, D))], axis=1)


def _plan():
    jobs = []
    for part in range(F // 256):
        jobs += [("gu_b", part)] + [("gu_a", part, t) for t in range(4)]
        if part in (2, 4):
            jobs += [("down", part // 2 - 1, n) for n in range(5)]
    jobs += [("down", 2, n) for n in range(5)] + [("oproj", n) for n in range(5)]
    jobs[2:2] = [("olast", 0), ("olast", 1)]
    jobs, tail = jobs[:-AHEAD], jobs[-AHEAD:]
    slot = {1 + (j + 1) * (NSTEP - 3) // len(jobs): job for j, job in enumerate(jobs)}
    seq = []
    for i in range(1, NSTEP + AHEAD):
        seq.append(("qk", i) if i < NSTEP else tail[i - NSTEP])
        if i in slot:
            seq.append(slot[i])
        if i >= AHEAD:
            seq.append(("pv", i - AHEAD))

    def time_line():
        events, now, t_scored = [], 0, {}
        for job in seq:
            if job[0] == "pv":
                now = max(now, t_scored.get(job[1], -T) + LEAD + 1)
            rows = T - nv[job[1]] if job[0] == "qk" else VR if job[0] == "pv" else T
            cycles = rows // 4 if job == ("olast", 1) else rows
            step = 8 if job[0] == "pv" else 16
            events += [(now + r * cycles // rows, ("lhs", job, r)) for r in range(0, rows, step)]
            events.append((now + (rows - step) * cycles // rows, ("dot", job)))
            for r in range(0, rows, step):
                t = now + r + step - 8 + LAT + SLACK
                events += [(t - 32, ("pre", job, r)), (t, ("res", job, r))]
            if job[0] == "qk":
                t_scored[job[1]] = t
            elif job[0] == "pv":
                events += [(now - LEAD + 8 * u, ("p_load", job[1], 3 - u)) for u in range(4)]
                s, c = divmod(job[1], NB)
                if c == NB - 1:
                    events.append((t + 8 if s < NSET - 1 else 24, ("norm", s)))
                    events += [(now + rows + LAT + 320, ("o_tile", kt)) for kt in range(4)
                               if (T * kt + T - 1) // (4 * DH) == s]
            now += cycles
        events += [(320, ("o_tile", 4)), (-100, ("q_stage",))]
        events += [(40 + 32 * n, ("x_stage", kt)) for n, kt in enumerate((4, 0, 1, 2, 3, 5, 6))]
        return events + [(64 * s, ("q_pin", s)) for s in range(1, NSET)]

    def alu_ops(ev):
        if ev[0] == "res":
            return {"qk": 12, "pv": 4, "gu_a": 11, "gu_b": 0, "down": 8, "oproj": 10,
                    "olast": 4 if ev[1][1] else 16}[ev[1][0]]
        return {"norm": 110, "o_tile": 24, "x_stage": 8}.get(ev[0], 0)

    nv, scoring, t_free = [NV] * NSTEP, [], 70
    for i in range(1, NSTEP):
        events = time_line()
        t_load = {ev[1:]: t for t, ev in events if ev[0] == "p_load"}
        other = sorted((t, alu_ops(ev)) for t, ev in events if alu_ops(ev))
        t = max(t_free, t_load[i - NP, 0] + 16) if i > NP else t_free
        halves = []
        for u in range(8):
            t_end = t + (86 if u % 2 else 76) / RATE
            for t_op, n in other:
                if t < t_op <= t_end:
                    t_end += n / RATE
            t = t_end
            halves.append((t - (0 if u % 2 else 12), ("score", i, u)))
        if t <= t_load[i, 3] - 8:
            scoring, t_free = scoring + halves, t
        else:
            nv[i] = 0

    def order(e):
        return e[0] // 16, e[1][0] in ("lhs", "dot", "p_load", "pre"), e[0]

    return [ev for _, ev in sorted(time_line() + scoring, key=order)], nv


def _kernel(x_hbm, wq_hbm, wkt_hbm, wvt_hbm, wo_hbm, wg_hbm, wu_hbm, wd_hbm, gw_hbm, out_hbm,
            x_v, wq_v, wo_v, wg_v, wu_v, wd_v, wkt_v, wvt_v, gw_v,
            qt_v, q_v, kb_v, p0_v, sp_v, g_v, omg_v, ot_v, out_v, in_sem, out_sem):
    def ld(rc, rows, lanes=T):
        return sp_v[rc[0]:rc[0] + rows, rc[1]:rc[1] + lanes]

    def rows_of(src, dst, r0, n):
        return src.at[pl.ds(r0, n)], dst.bitcast(BF).at[pl.ds(r0, n)]

    pairs = [rows_of(x_hbm, x_v, *X_SPANS[0]), (wkt_hbm, wkt_v), (wvt_hbm, wvt_v), (gw_hbm, gw_v),
             rows_of(wq_hbm, wq_v, 512, T), rows_of(wq_hbm, wq_v, 0, 512)]
    pairs += [rows_of(x_hbm, x_v, *span) for span in X_SPANS[1:]]
    pairs += [(src, dst.bitcast(BF)) for src, dst in
              ((wg_hbm, wg_v), (wu_hbm, wu_v), (wd_hbm, wd_v), (wo_hbm, wo_v))]
    copies = [pltpu.make_async_copy(src, dst, in_sem.at[i]) for i, (src, dst) in enumerate(pairs)]
    for copy in copies:
        copy.start()
    sp_v[A0:A0 + 2 * T, :] = jnp.zeros((2 * T, 4 * T), F32)
    sp_v[PV0:PV0 + VR, :] = jnp.ones((VR, 4 * T), F32)
    ot_v[4 * T:5 * T, :] = jnp.zeros((T, T), F32)
    for copy in copies[:5]:
        copy.wait()

    pad = jnp.zeros((4, D), F32)
    wkv = jnp.concatenate(
        [wkt_v[...].astype(F32), pad, wvt_v[...].astype(F32),
         gw_v[...].astype(F32).reshape(1, D), pad[0:3]], axis=0).astype(BF)
    row = lax.broadcasted_iota(jnp.int32, (VR, T), 0)

    def project_kv(m0, n):
        kv = lax.dot_general(wkv, _unpack(x_v, m0, m0 + n, 0, D), (((1,), (1,)), ((), ())),
                             preferred_element_type=F32)
        for c in range(m0 // T, (m0 + n) // T):
            kvc = kv[:, c * T - m0:(c + 1) * T - m0]
            k = jnp.concatenate([_round(kvc[0:VR]), jnp.zeros((T - VR, T), F32)], axis=0).T
            r, l = _at(K0, 64, c)
            sp_v[r:r + 64, l:l + T] = pltpu.bitcast(k.astype(BF), F32)
            kb = [[jnp.stack([jnp.broadcast_to(k[j:j + 16, d:d + 1], (16, T))
                              for d in range(d0, d0 + HD)]) for d0 in (0, HD)]
                  for j in (T - NV, T - NV // 2)]
            for u in range(8):
                kb_v[c, u] = kb[VPU_BLOCKS[u // 2][0]][u % 2]
            r, l = _at(V0, VR, c)
            sp_v[r:r + VR, l:l + T] = jnp.where(
                row < DH, _round(kvc[VR:2 * VR]), jnp.where(row == DH, 1.0, 0.0))
            g = jax.nn.sigmoid(kvc[VR + DH:VR + DH + 1])
            g_v[c] = jnp.broadcast_to(g, (8, T))
            omg_v[c] = jnp.broadcast_to(1.0 - g, (T, T)).T

    def store_q(b0, q):
        for b in (b0, b0 + 1):
            qt = _round(q[(b - b0) * T:(b - b0 + 1) * T] * QSCALE).T
            qt = jnp.concatenate([qt, jnp.zeros((8, T), F32)], axis=0)
            for h in range(H):
                qt_v[h // 4][b * VR:(b + 1) * VR, (h % 4) * T:(h % 4 + 1) * T] = (
                    qt[h * DH:h * DH + VR])

    def first_tile(b):
        k = pltpu.bitcast(ld(_at(K0, 64, 0), 64), BF)[:, 0:VR]
        p = jnp.exp2(_dot(k, qt_v[0][b * VR:(b + 1) * VR, :]))
        p0_v[b] = pltpu.bitcast(p.astype(BF), F32)

    pending, b_next = None, 0
    for i, (m0, n) in enumerate(X_SPANS):
        if i > 0:
            copies[5 + i].wait()
        project_kv(m0, n)
        for m in range(m0, m0 + n, 2 * T):
            y = _last_rows_dot(_unpack(x_v, m, m + 2 * T, 512, D), wq_v)
            if m == 0:
                copies[5].wait()
            q = jnp.concatenate(
                [_dot(_unpack(x_v, m, m + 2 * T, 0, 512), _unpack(wq_v, 0, 512, j * T, (j + 1) * T))
                 + y[:, j * T:(j + 1) * T] for j in range(5)], axis=1)
            if pending:
                store_q(*pending)
            pending = m // T, q
            for b in range(b_next, min(b_next + 2, m0 // T - 2)):
                first_tile(b)
                b_next = b + 1
    store_q(*pending)
    for b in range(b_next, NB):
        first_tile(b)
    for copy in copies[-4:]:
        copy.wait()

    def head_set(s, b):
        return qt_v[s][pl.ds(pl.multiple_of(b * VR, 8), VR), :]

    def normalize(s, acc, b):
        g = g_v[b, 0:1, :]
        sums = []
        for t in range(4):
            a = acc[:, t * T:(t + 1) * T]
            sums.append(a[DH:DH + 1])
            ot_v[(4 * s + t) * DH:(4 * s + t + 1) * DH, :] = a[0:DH] * (g * pl.reciprocal(sums[t]))
        return sums

    def widen(bounds, sums):
        for l in sums:
            bounds = jnp.minimum(bounds[0], l), jnp.maximum(bounds[1], l)
        return bounds

    def out_copy(r0, sem):
        return pltpu.make_async_copy(out_v.at[pl.ds(r0 + T, T)], out_hbm.at[pl.ds(r0, T)], sem)

    events, nv = _plan()

    def block(b, bounds):
        zero = pl.multiple_of(lax.shift_right_logical(b, 16) * 8, 8)
        vals, ready = {}, set()

        def put(rc, val):
            if val.dtype == BF:
                val = pltpu.bitcast(val, F32)
            sp_v[pl.ds(zero + rc[0], val.shape[0]), rc[1]:rc[1] + val.shape[1]] = val

        def p_at(i, t, key):
            return _at(P0, 64, (i % NP) * 4 + t, key // 2)

        def score(i, u):
            s, c = divmod(i, NB)
            half, t0 = VPU_BLOCKS[u // 2]
            d0 = half * VR + (u % 2) * HD
            q = [jnp.concatenate(
                [jnp.broadcast_to(q_v[s][d:d + 1, t * T:(t + 1) * T], (16, T))
                 for t in (t0, t0 + 1)], axis=1) for d in range(d0, d0 + HD)]
            y = vals.pop("score", None)
            for d in range(HD):
                k = kb_v[c, u, d]
                term = jnp.concatenate([k, k], axis=1) * q[d]
                y = term if y is None else y + term
            if u % 2 == 0:
                vals["score"] = y
                put((J0, 0), y)
            else:
                assert i <= NP or ("p_load", i - NP, 0) in ready
                put(p_at(i, t0, T - NV + 16 * half), jnp.exp2(y).astype(BF))
                ready.add(("score", i, u))

        def q_stage():
            for s in range(NSET):
                q = head_set(s, b)
                q_v[s][0:VR, :] = q
                q_v[s][VR:2 * VR, :] = q

        def q_pin(s):
            put((J0, 2 * T), q_v[s][2 * VR - 8:2 * VR, 3 * T:4 * T])

        def x_stage(kt):
            if kt < 5:
                val = x_v[pl.ds(pl.multiple_of(b * 64, 64), 64), kt * T:(kt + 1) * T]
            else:
                val = omg_v[b, (kt - 5) * 64:(kt - 4) * 64, :]
            put(_at(X0, 64, kt), val)
            ready.update((X0, kt, r) for r in range(0, T, 16))

        def p_load(i, u):
            if i == 0:
                val = p0_v[b, 16 * u:16 * (u + 1), :]
            else:
                assert ("qk", i, T - nv[i] - 16) in ready
                assert not nv[i] or ("score", i, 7) in ready
                val = ld(p_at(i, 0, 32 * u), 16, 4 * T)
            vals.setdefault(("p", i), []).insert(0, val)
            ready.add(("p_load", i, u))

        def lhs(job, r):
            if job[0] == "qk":
                val = ld(_at(K0, 64, job[1] % NB, r // 2), 8)
            elif job[0] == "pv":
                val = ld(_at(V0, VR, job[1] % NB, r), 8)
            else:
                base, kt, n = {"gu_b": (X0, 4, 1), "gu_a": (X0, 0, 4), "down": (H0, 4 * job[1], 4),
                               "oproj": (O0, 0, 4), "olast": (O0, 4, 1)}[job[0]]
                assert all((base, kt + j, r) in ready for j in range(n))
                val = ld(_at(base, 64, kt, r // 2), 8, n * T)
            vals.setdefault(("lhs", job), []).append(val)

        def dot(job):
            a = jnp.concatenate(vals.pop(("lhs", job)), axis=0)
            if job[0] == "pv":
                w = pltpu.bitcast(jnp.concatenate(vals.pop(("p", job[1])), axis=0), BF)
            else:
                a = pltpu.bitcast(a, BF)
            if job[0] == "qk":
                a, w = a[:, 0:VR], q_v[job[1] // NB][0:VR, :]
            elif job[0] == "gu_b":
                c0 = job[1] * 256
                w = pltpu.bitcast(jnp.concatenate(
                    [wg_v[256:320, c0:c0 + 256], wu_v[256:320, c0:c0 + 256]], axis=1), BF)
            elif job[0] == "gu_a":
                c0 = job[1] * 256 + (job[2] // 2) * T
                w = _unpack((wg_v, wu_v)[job[2] % 2], 0, 512, c0, c0 + T)
            elif job[0] == "down":
                w = _unpack(wd_v, job[1] * 512, (job[1] + 1) * 512, job[2] * T, (job[2] + 1) * T)
            elif job[0] == "oproj":
                w = _unpack(wo_v, 0, 512, job[1] * T, (job[1] + 1) * T)
            elif job[0] == "olast":
                w = _unpack(wo_v, 512, D, (0, 512)[job[1]], (512, D)[job[1]])
            vals["y", job] = _quarters(a, w) if job == ("olast", 1) else _dot(a, w)

        def pre(job, r):
            if job[0] == "gu_a":
                up, j = job[2] % 2, job[2] // 2
                src = [_at(G0, T, 2 * up + j, r)] + [_at(G0, T, j, r)] * up
            elif job[0] == "olast":
                src = [_at(A0, T, n, r) for n in ((0, 1, 2, 3), (4,))[job[1]]]
            elif job[0] == "oproj" or (job[0] == "down" and job[1] > 0):
                src = [_at(A0, T, job[-1], r)]
            else:
                src = []
            assert job[0] == "olast" or all(rc in ready for rc in src)
            ready.difference_update(src)
            if job[0] == "oproj":
                src.append(_at(X0, 64, 5 + r // 64, r % 64))
            vals["pre", job, r] = [ld(rc, 16) for rc in src]

        def res(job, r):
            y = vals["y", job][r:r + (8 if job[0] == "pv" else 16)]
            old = vals.pop(("pre", job, r))
            if job[0] == "qk":
                assert job[1] <= NP or ("p_load", job[1] - NP, 0) in ready
                put(p_at(job[1], 0, r), jnp.exp2(y).astype(BF))
                ready.add(("qk", job[1], r))
            elif job[0] == "pv":
                vals["pv", r] = y = y + vals["pv", r] if job[1] % NB else y
                if job[1] == NSTEP - 1:
                    put((PV0 + r, 0), y)
                elif job[1] % NB == NB - 1:
                    vals.setdefault("acc", []).append(y)
            elif job[0] == "gu_b":
                put((G0 + r, 0), y)
                ready.update(_at(G0, T, j, r) for j in range(4))
            elif job[0] == "gu_a":
                up, j = job[2] % 2, job[2] // 2
                y = y + old[0]
                if up:
                    put(_at(H0, 64, 2 * job[1] + j, r // 2), (old[1] * y).astype(BF))
                    ready.add((H0, 2 * job[1] + j, r))
                else:
                    put(_at(G0, T, j, r), jnp.maximum(y, 0.0))
                    ready.add(_at(G0, T, j, r))
            elif job[0] == "olast":
                r0 = pl.multiple_of(b * T + r, 16)
                for j, n in enumerate(((0, 1, 2, 3), (4,))[job[1]]):
                    out_v[pl.ds(r0, 16), n * T:(n + 1) * T] = (
                        y[:, j * T:(j + 1) * T] + old[j]).astype(BF)
            else:
                if job[0] == "oproj":
                    old = [old[0] * old[1]]
                put(_at(A0, T, job[-1], r), y + old[0] if old else y)
                ready.add(_at(A0, T, job[-1], r))

        def norm(s):
            if s < NSET - 1:
                sums = normalize(s, jnp.concatenate(vals.pop("acc"), axis=0), b)
            else:
                sums = normalize(s, ld((PV0, 0), VR, 4 * T), jnp.maximum(b - 1, 0))
            vals["bounds"] = widen(vals["bounds"], sums)

        def o_tile(kt):
            put(_at(O0, 64, kt), ot_v[kt * T:(kt + 1) * T, :].T.astype(BF))
            ready.update((O0, kt, r) for r in range(0, T, 16))

        emit = dict(score=score, q_stage=q_stage, q_pin=q_pin, x_stage=x_stage, p_load=p_load,
                    lhs=lhs, dot=dot, pre=pre, res=res, norm=norm, o_tile=o_tile)
        vals["bounds"] = bounds
        for kind, *args in events:
            emit[kind](*args)

        @pl.when(b > 0)
        def _():
            out_copy(pl.multiple_of((b - 1) * T, T), out_sem.at[b - 1]).start()

        return vals["bounds"]

    bounds = lax.fori_loop(0, NB, block, (jnp.ones((1, T), F32), jnp.ones((1, T), F32)))
    bounds = widen(bounds, normalize(NSET - 1, ld((PV0, 0), VR, 4 * T), NB - 1))
    last = _last_rows_dot(ot_v[4 * T:5 * T, :].T.astype(BF), wo_v)
    last += jnp.concatenate([ld((A0, 0), T, 4 * T), ld((A0 + T, 0), T)], axis=1)
    out_v[S:S + T, :] = last.astype(BF)
    out_copy(S - T, out_sem.at[NB - 1]).start()
    safe = ((jnp.min(bounds[0]) >= L_LO) & (jnp.max(bounds[1]) <= L_HI)
            & (jnp.max(jnp.abs(ld((V0, 0), 4 * VR, 4 * T))) <= V_HI))
    for b in range(NB):
        out_copy(b * T, out_sem.at[b]).wait()

    @pl.when(jnp.logical_not(safe))
    def _():
        @pl.loop(0, NB)
        def _(b):
            for s in range(NSET):
                q = head_set(s, b)

                def chunk(c, carry):
                    m_old, acc = carry
                    lanes = pl.ds(pl.multiple_of((c % 4) * T, T), T)
                    k = sp_v[pl.ds(pl.multiple_of(K0 + (c // 4) * 64, 8), 64), lanes]
                    v = sp_v[pl.ds(pl.multiple_of(V0 + (c // 4) * VR, 8), VR), lanes]
                    y = _dot(pltpu.bitcast(k, BF)[:, 0:VR], q)
                    m_new = jnp.maximum(m_old, jnp.max(y, axis=0, keepdims=True))
                    p = jnp.exp2(y - m_new).astype(BF)
                    return m_new, _dot(v, p) + acc * jnp.exp2(m_old - m_new)

                init = jnp.full((1, 4 * T), -3.4e38, F32), jnp.zeros((VR, 4 * T), F32)
                normalize(s, lax.fori_loop(0, NB, chunk, init)[1], b)
            x = pltpu.bitcast(x_v[pl.ds(pl.multiple_of(b * 64, 64), 64), :], BF)
            h = (jnp.maximum(_dot(x, _unpack(wg_v, 0, D, 0, F)), 0.0)
                 * _dot(x, _unpack(wu_v, 0, D, 0, F)))
            y = (jnp.concatenate([omg_v[b]] * 5, axis=1)
                 * _dot(h.astype(BF), _unpack(wd_v, 0, F, 0, D)))
            y += _dot(ot_v[...].T.astype(BF), _unpack(wo_v, 0, D, 0, D))
            out_v[pl.ds(pl.multiple_of(b * T, T), T), :] = y.astype(BF)

        copy = pltpu.make_async_copy(out_v.at[pl.ds(0, S)], out_hbm, out_sem.at[0])
        copy.start()
        copy.wait()


@jax.jit
def pallas_gated_mix__grouped_kv_mqa__glu_gated_reglu__prompt_kernel(
    A_x: jax.Array,
    A_wq: jax.Array,
    A_wk: jax.Array,
    A_wv: jax.Array,
    A_wo: jax.Array,
    B_x: jax.Array,
    B_W_gate: jax.Array,
    B_W_up: jax.Array,
    B_W_down: jax.Array,
    gate_w: jax.Array,
):
    del B_x
    hbm = pl.BlockSpec(memory_space=pl.ANY)
    out = pl.pallas_call(
        _kernel,
        out_shape=jax.ShapeDtypeStruct((S, D), BF),
        in_specs=[hbm] * 9,
        out_specs=hbm,
        scratch_shapes=[
            pltpu.VMEM((S // 2, D), F32),
            pltpu.VMEM((D // 2, D), F32),
            pltpu.VMEM((D // 2, D), F32),
            pltpu.VMEM((D // 2, F), F32),
            pltpu.VMEM((D // 2, F), F32),
            pltpu.VMEM((F // 2, D), F32),
            pltpu.VMEM((DH, D), BF),
            pltpu.VMEM((DH, D), BF),
            pltpu.VMEM((D,), BF),
            [pltpu.VMEM((NB * VR, 4 * T), F32)] * NSET,
            [pltpu.VMEM((2 * VR, 4 * T), F32)] * NSET,
            pltpu.VMEM((NB, 8, HD, 16, T), F32),
            pltpu.VMEM((NB, 64, 4 * T), F32),
            pltpu.VMEM((SP_ROWS, 4 * T), F32),
            pltpu.VMEM((NB, 8, T), F32),
            pltpu.VMEM((NB, T, T), F32),
            pltpu.VMEM((D, T), F32),
            pltpu.VMEM((S + T, D), BF),
            pltpu.SemaphoreType.DMA((9 + len(X_SPANS),)),
            pltpu.SemaphoreType.DMA((NB,)),
        ],
        compiler_params=pltpu.CompilerParams(vmem_limit_bytes=64 * 2 ** 20),
        name="gated_mix_mqa_reglu",
    )(A_x.reshape(S, D), A_wq, A_wk.T, A_wv.T, A_wo, B_W_gate, B_W_up, B_W_down, gate_w)
    return out.reshape(1, S, D)
```
